```python
import jax
import jax.numpy as jnp

def _softmax(x, axis=-1):
    return jax.nn.softmax(x, axis=axis)
def _gelu(x):
    return jax.nn.gelu(x, approximate=True)
def _silu(x):
    return jax.nn.silu(x)
def _sigmoid(x):
    return jax.nn.sigmoid(x)
def _layernorm(x, axis=-1, eps=1e-5):
    m = jnp.mean(x, axis=axis, keepdims=True)
    v = jnp.var(x, axis=axis, keepdims=True)
    return (x - m) / jnp.sqrt(v + eps)
def _scatter_add(tgt, idx, src, axis=0):
    return tgt.at[idx].add(src)
def _segment_sum(src, seg, n):
    return jax.ops.segment_sum(src, seg, n)
class _Rng:
    def __init__(self, key):
        self._k = key
    def _next(self):
        self._k, sub = jax.random.split(self._k)
        return sub
    def normal(self, shape):
        return jax.random.normal(self._next(), shape, dtype=jnp.bfloat16)
    def randint(self, lo, hi, shape):
        return jax.random.randint(self._next(), shape, lo, hi, dtype=jnp.int32)
    def uniform(self, shape, lo=0.0, hi=1.0):
        return jax.random.uniform(self._next(), shape, jnp.bfloat16, lo, hi)
    def permutation(self, n):
        return jax.random.permutation(self._next(), n)


kernel_name = 'parallel_sum__sliding_local_dilated__mixer_token_mlp__prompt'

def setup_inputs():
    _rng = _Rng(jax.random.key(int.from_bytes(__import__("os").urandom(4), "little")))
    _w = (lambda a: (lambda t: t.astype(jnp.bfloat16) if jnp.issubdtype(t.dtype, jnp.floating) else t)(jnp.asarray(a)))
    def _A_setup():
        B, S, D = 1, 2048, 448
        return {
            "x": _w((lambda *s: _rng.normal(s) * 0.05)(B, S, D)),
            "wqkv": _w((lambda *s: _rng.normal(s) * 0.05)(D, 3 * D)),
            "wo": _w((lambda *s: _rng.normal(s) * 0.05)(D, D)),
        }
    _A_in = _A_setup()

    def _B_setup():
        B, S, D, F = 1, 2048, 448, 1792
        return {
            "x": _w((lambda *s: _rng.normal(s) * 0.05)(B, S, D)),
            "w1": _w((lambda *s: _rng.normal(s) * 0.05)(S, F) * (S ** -0.5)),
            "b1": _w((lambda *s: _rng.normal(s) * 0.05)(F) * 0.02),
            "w2": _w((lambda *s: _rng.normal(s) * 0.05)(F, S) * (F ** -0.5)),
            "b2": _w((lambda *s: _rng.normal(s) * 0.05)(S) * 0.02),
        }
    _B_in = _B_setup()

    return {
        "A_x": _A_in["x"],
        "A_wqkv": _A_in["wqkv"],
        "A_wo": _A_in["wo"],
        "B_x": _B_in["x"],
        "B_w1": _B_in["w1"],
        "B_b1": _B_in["b1"],
        "B_w2": _B_in["w2"],
        "B_b2": _B_in["b2"],
    }

def reference(A_x, A_wqkv, A_wo, B_x, B_w1, B_b1, B_w2, B_b2):
    def _A_ref(x, wqkv, wo):
        B, S, D = x.shape
        H = 16; Dh = D // H
        W, dil = 8, 2
        qkv = (lambda x, *d: x.transpose(*d))((x @ wqkv).reshape(B, S, 3, H, Dh), 2, 0, 3, 1, 4)
        q, k, v = qkv[0], qkv[1], qkv[2]
        scale = Dh ** -0.5
        pos = jnp.arange(S)
        off = jnp.arange(W) * dil
        idx = pos[:, None] - off[None, :]
        mask = idx >= 0
        idx_c = jnp.where(mask, idx, 0).reshape(-1)
        kg = k[:, :, idx_c, :].reshape(B, H, S, W, Dh)
        vg = v[:, :, idx_c, :].reshape(B, H, S, W, Dh)
        logits = jnp.einsum("bhsd,bhswd->bhsw", q, kg) * scale
        logits = jnp.where(mask[None, None, :, :], logits, -1e9)
        attn = _softmax(logits, axis=-1)
        o = jnp.einsum("bhsw,bhswd->bhsd", attn, vg)
        return (lambda x, *d: x.transpose(*d))(o, 0, 2, 1, 3).reshape(B, S, D) @ wo

    def _B_ref(x, w1, b1, w2, b2):
        B, S, D = x.shape
        h = _layernorm(x, axis=-1)
        u = jnp.einsum("bsd,sf->bdf", h, w1) + b1
        u = _gelu(u)
        y = jnp.einsum("bdf,fs->bds", u, w2) + b2
        return (lambda x, *d: x.transpose(*d))(y, 0, 2, 1)

    x = A_x
    xn = _layernorm(x, axis=-1)
    return x + _A_ref(xn, A_wqkv, A_wo) + _B_ref(xn, B_w1, B_b1, B_w2, B_b2)
```

```python
import jax
import jax.numpy as jnp
import jax.experimental.pallas as pl
import jax.experimental.pallas.tpu as pltpu

_S, _D, _F = 2048, 448, 1792
_H, _DH = 16, 28
_W, _DIL = 8, 2
_T = 128
_NT = _S // _T
_NF = _F // _T
_EPS = 1e-5
_CHUNKS = ((0, 1), (1, 2), (2, 4), (4, 8), (8, 12), (12, 16))

_f32, _bf16, _u32 = jnp.float32, jnp.bfloat16, jnp.uint32


def _ln_t(x):
    m = jnp.sum(x, axis=0, keepdims=True) * (1.0 / _D)
    c = x - m
    v = jnp.sum(c * c, axis=0, keepdims=True) * (1.0 / _D)
    return c * jax.lax.rsqrt(v + _EPS)


def _gelu(z):
    inner = 0.7978845608028654 * (z + 0.044715 * (z * z * z))
    return 0.5 * z * (1.0 + jnp.tanh(inner))


def _pack(x):
    return pltpu.bitcast(x.astype(_bf16), _u32)


def _unpack(x):
    return pltpu.bitcast(x, _bf16).astype(_f32)


def _kernel(xt_hbm, wqkv_hbm, wo_hbm, w1_hbm, b1_hbm, w2_hbm, b2_hbm, out_hbm,
            xt_v, wqkv_v, wo_v, w1_v, b1_v, w2_v, b2_v,
            xnt_s, ht_s, uacc, u_s, wt_s, wot_s, perm_s, perm2_s,
            qt_s, kp_s, vp_s, ot_s, out_v,
            sem_x, sem_w1, sem_w2, sem_misc, sem_out, sem_f):
    tile = lambda p: slice(p * _T, (p + 1) * _T)
    n_ch = len(_CHUNKS)
    cols = lambda a, b: slice(a * _T, b * _T)

    x_parts = ((0, 2), (2, 16))
    cp_x = [pltpu.make_async_copy(xt_hbm.at[:, cols(a, b)], xt_v.at[:, cols(a, b)], sem_x.at[i])
            for i, (a, b) in enumerate(x_parts)]
    cp_w1 = [pltpu.make_async_copy(w1_hbm.at[cols(a, b)], w1_v.at[cols(a, b)], sem_w1.at[i])
             for i, (a, b) in enumerate(_CHUNKS)]
    w2_parts = ((0, 8), (8, 16))
    cp_w2 = [pltpu.make_async_copy(w2_hbm.at[:, cols(a, b)], w2_v.at[:, cols(a, b)], sem_w2.at[i])
             for i, (a, b) in enumerate(w2_parts)]
    cp_wqkv = pltpu.make_async_copy(wqkv_hbm, wqkv_v, sem_misc.at[0])
    cp_wo = pltpu.make_async_copy(wo_hbm, wo_v, sem_misc.at[1])
    cp_b1 = pltpu.make_async_copy(b1_hbm, b1_v, sem_misc.at[2])
    cp_b2 = pltpu.make_async_copy(b2_hbm, b2_v, sem_misc.at[3])
    out_parts = ((0, 8), (8, 15), (15, 16))
    cp_out = [pltpu.make_async_copy(out_v.at[:, cols(a, b)], out_hbm.at[:, cols(a, b)], sem_out.at[i])
              for i, (a, b) in enumerate(out_parts)]

    def layernorms(p):
        x = xt_v[:, tile(p)].astype(_f32)
        xn = _ln_t(x)
        xnt_s[:, tile(p)] = pltpu.bitcast(xn.astype(_bf16), _u32)
        ht_s[:, tile(p)] = _ln_t(xn).astype(_bf16)

    def prep_wqkv():
        for c in range((3 * _D + _T - 1) // _T):
            lo, hi = c * _T, min((c + 1) * _T, 3 * _D)
            blk = wqkv_v[:, lo:hi].T.astype(_f32)
            for j in range(4):
                l, h = j * _T, min((j + 1) * _T, _D)
                perm_s[j, lo:hi, 0:h - l] = blk[:, l:h]
        for t in range(3):
            for d in range(_DH):
                r0 = t * _D + d * _H
                for j in range(4):
                    l, h = j * _T, min((j + 1) * _T, _D)
                    g = perm_s[j, pl.ds(t * _D + d, _H, stride=_DH), :]
                    wt_s[r0:r0 + _H, l:h] = g[:, 0:h - l].astype(_bf16)

    def prep_wo():
        for j in range(4):
            l, h = j * _T, min((j + 1) * _T, _D)
            perm2_s[j, :, 0:h - l] = wo_v[:, l:h].astype(_f32)
        for j in range(4):
            l, h = j * _T, min((j + 1) * _T, _D)
            g = jnp.concatenate(
                [perm2_s[j, pl.ds(d, _H, stride=_DH), :] for d in range(_DH)], axis=0)
            wot_s[l:h, :] = g[:, 0:h - l].astype(_bf16).T

    def mix1(c, f):
        k0, k1 = _CHUNKS[c][0] * _T, _CHUNKS[c][1] * _T
        r = jnp.dot(ht_s[:, k0:k1], w1_v[k0:k1, tile(f)], preferred_element_type=_f32)
        if c == 0:
            uacc[:, tile(f)] = r
        elif c < n_ch - 1:
            uacc[:, tile(f)] += r
        else:
            b = b1_v[pl.ds(f * _T, _T)].astype(_f32).reshape(1, _T)
            u_s[:, tile(f)] = _gelu(uacc[:, tile(f)] + r + b).astype(_bf16)

    def qkv(p):
        xn = pltpu.bitcast(xnt_s[:, tile(p)], _bf16)
        qt_s[:, tile(p)] = jnp.dot(wt_s[0:_D, :], xn, preferred_element_type=_f32)
        kp_s[:, tile(p)] = _pack(jnp.dot(wt_s[_D:2 * _D, :], xn, preferred_element_type=_f32))
        vp_s[:, tile(p)] = _pack(jnp.dot(wt_s[2 * _D:3 * _D, :], xn, preferred_element_type=_f32))

    lane = jax.lax.broadcasted_iota(jnp.int32, (8, _T), 1)
    lane16 = jax.lax.broadcasted_iota(jnp.int32, (_H, _T), 1)

    def shifted(ref, p, d, w):
        cur = ref[d * 8:(d + 1) * 8, tile(p)]
        sh = _DIL * w
        if w > 0:
            if p > 0:
                prev = ref[d * 8:(d + 1) * 8, tile(p - 1)]
                cur = jnp.where(lane >= _T - sh, prev, cur)
            cur = pltpu.roll(cur, sh, 1)
        return _unpack(cur)

    def attention(p):
        lg = [None] * _W
        for d in range(_DH):
            q = qt_s[d * _H:(d + 1) * _H, tile(p)]
            for w in range(_W):
                t = q * shifted(kp_s, p, d, w)
                lg[w] = t if lg[w] is None else lg[w] + t
        scale = _DH ** -0.5
        for w in range(_W):
            lg[w] = lg[w] * scale
            if p == 0 and w > 0:
                lg[w] = jnp.where(lane16 >= _DIL * w, lg[w], -1e9)
        m = lg[0]
        for w in range(1, _W):
            m = jnp.maximum(m, lg[w])
        e = [jnp.exp(lg[w] - m) for w in range(_W)]
        s = e[0]
        for w in range(1, _W):
            s = s + e[w]
        r = 1.0 / s
        a = [e[w] * r for w in range(_W)]
        for d in range(_DH):
            acc = None
            for w in range(_W):
                t = a[w] * shifted(vp_s, p, d, w)
                acc = t if acc is None else acc + t
            ot_s[d * _H:(d + 1) * _H, tile(p)] = acc.astype(_bf16)

    def finish(p):
        y = jnp.dot(u_s[...], w2_v[:, tile(p)], preferred_element_type=_f32)
        a = jnp.dot(wot_s[...], ot_s[:, tile(p)], preferred_element_type=_f32)
        b = b2_v[pl.ds(p * _T, _T)].astype(_f32).reshape(1, _T)
        res = (xt_v[:, tile(p)].astype(_f32) + a) + (y + b)
        out_v[:, tile(p)] = res.astype(_bf16)

    def fence():
        pl.semaphore_signal(sem_f, 1)
        pl.semaphore_wait(sem_f, 1)
    order = [cp_x[0], cp_w1[0], cp_x[1], cp_w1[1], cp_w1[2], cp_w1[3], cp_wqkv, cp_wo, cp_b1, cp_b2, cp_w1[4], cp_w1[5], cp_w2[0], cp_w2[1]]
    for c in order:
        c.start()
        fence()

    cp_x[0].wait(); cp_w1[0].wait()
    layernorms(0)
    ln_todo = list(range(1, _NT))
    ln_plan = {0: 1, 1: 2, 2: 4, 3: 8}
    for c in range(n_ch):
        if c == 1:
            cp_x[1].wait()
        if c >= 1:
            cp_w1[c].wait()
        if c == 4:
            cp_wqkv.wait(); cp_wo.wait(); cp_b1.wait(); cp_b2.wait()
        n_ln = ln_plan.get(c, 0)
        for f in range(_NF):
            mix1(c, f)
            while n_ln and (f + 1) * ln_plan.get(c, 0) >= (ln_plan.get(c, 0) - n_ln + 1) * _NF - 0:
                layernorms(ln_todo.pop(0)); n_ln -= 1
            if c == 4 and f == 2:
                prep_wqkv()
            if c == 4 and f == 9:
                prep_wo()
            if c == 5 and f == 6:
                qkv(0)
            if c == 5 and f == 10:
                qkv(1)
    assert not ln_todo

    cp_w2[0].wait()
    attention(0)
    for p in range(_NT):
        if p + 2 < _NT:
            qkv(p + 2)
        if p + 1 < _NT:
            attention(p + 1)
        finish(p)
        if p == 5:
            cp_w2[1].wait()
        if p == 7:
            cp_out[0].start()
        if p == 14:
            cp_out[1].start()
    cp_out[2].start()
    for c in cp_out:
        c.wait()


@jax.jit
def pallas_parallel_sum__sliding_local_dilated__mixer_token_mlp__prompt_kernel(
    A_x, A_wqkv, A_wo, B_x, B_w1, B_b1, B_w2, B_b2,
):
    del B_x
    n_ch = len(_CHUNKS)
    scratch = [
        pltpu.VMEM((_D, _S), _bf16),
        pltpu.VMEM((_D, 3 * _D), _bf16),
        pltpu.VMEM((_D, _D), _bf16),
        pltpu.VMEM((_S, _F), _bf16),
        pltpu.VMEM((_F,), _bf16),
        pltpu.VMEM((_F, _S), _bf16),
        pltpu.VMEM((_S,), _bf16),
        pltpu.VMEM((_D // 2, _S), _u32),
        pltpu.VMEM((_D, _S), _bf16),
        pltpu.VMEM((_D, _F), _f32),
        pltpu.VMEM((_D, _F), _bf16),
        pltpu.VMEM((3 * _D, _D), _bf16),
        pltpu.VMEM((_D, _D), _bf16),
        pltpu.VMEM((4, 3 * _D, _T), _f32),
        pltpu.VMEM((4, _D, _T), _f32),
        pltpu.VMEM((_D, _S), _f32),
        pltpu.VMEM((_D // 2, _S), _u32),
        pltpu.VMEM((_D // 2, _S), _u32),
        pltpu.VMEM((_D, _S), _bf16),
        pltpu.VMEM((_D, _S), _bf16),
        pltpu.SemaphoreType.DMA((2,)),
        pltpu.SemaphoreType.DMA((n_ch,)),
        pltpu.SemaphoreType.DMA((2,)),
        pltpu.SemaphoreType.DMA((4,)),
        pltpu.SemaphoreType.DMA((3,)),
        pltpu.SemaphoreType.REGULAR,
    ]
    hbm = pl.BlockSpec(memory_space=pltpu.HBM)
    xt = jnp.swapaxes(A_x, 1, 2).reshape(_D, _S)
    out = pl.pallas_call(
        _kernel,
        out_shape=jax.ShapeDtypeStruct((_D, _S), _bf16),
        in_specs=[hbm] * 7,
        out_specs=hbm,
        scratch_shapes=scratch,
        compiler_params=pltpu.CompilerParams(vmem_limit_bytes=100 * 1024 * 1024),
    )(xt, A_wqkv, A_wo, B_w1, B_b1, B_w2, B_b2)
    return jnp.swapaxes(out.reshape(1, _D, _S), 1, 2)
```

```python
import jax
import jax.numpy as jnp
import jax.experimental.pallas as pl
import jax.experimental.pallas.tpu as pltpu

_S, _D, _F = 2048, 448, 1792
_H, _DH = 16, 28
_W, _DIL = 8, 2
_EPS = 1e-5
_T = 128
_NT = _S // _T
_NF = _F // _T
_DP = _D // 2

_f32, _bf16, _u32 = jnp.float32, jnp.bfloat16, jnp.uint32


def _ln_t(x):
    m = jnp.sum(x, axis=0, keepdims=True) * (1.0 / _D)
    c = x - m
    v = jnp.sum(c * c, axis=0, keepdims=True) * (1.0 / _D)
    return c * jax.lax.rsqrt(v + _EPS)


def _gelu(z):
    c0 = 0.7978845608028654
    inner = z * (c0 + (c0 * 0.044715) * (z * z))
    hz = 0.5 * z
    return hz + hz * jnp.tanh(inner)


def _pack(x):
    return pltpu.bitcast(x.astype(_bf16), _u32)


def _bf(x):
    return pltpu.bitcast(x, _bf16)


def _unpack(x):
    return _bf(x).astype(_f32)


def _dot(a, b):
    return jnp.dot(_bf(a), _bf(b), preferred_element_type=_f32)


def _kernel(xt_hbm, wqkv_hbm, wo_hbm, w1_hbm, b1_hbm, w2_hbm, b2_hbm, out_hbm,
            xt_v, wqkv_v, wo_v, w1_v, b1_v, w2_v, b2_v,
            xnt_s, ht_s, u_s, wt_s, wot_s, perm_s, perm2_s,
            qt_s, kp_s, vp_s, ot_s, out_v, y_s,
            sem_in, sem_out, sem_fence):
    def tile(p):
        return slice(p * _T, (p + 1) * _T)

    def cols(a, b):
        return slice(a * _T, b * _T)

    xt_hbm, wqkv_hbm, wo_hbm, w1_hbm, w2_hbm, out_hbm = (
        r.bitcast(_u32) for r in (xt_hbm, wqkv_hbm, wo_hbm, w1_hbm, w2_hbm, out_hbm))
    q_cols, kv_cols = slice(0, 4 * _T), slice(4 * _T, 3 * _D)
    loads = [
        (xt_hbm.at[:, cols(0, 4)], xt_v.at[:, cols(0, 4)]),
        (wqkv_hbm.at[:, q_cols], wqkv_v.at[:, q_cols]),
        (wqkv_hbm.at[:, kv_cols], wqkv_v.at[:, kv_cols]),
        (xt_hbm.at[:, cols(4, _NT)], xt_v.at[:, cols(4, _NT)]),
        (w1_hbm, w1_v), (wo_hbm, wo_v), (b1_hbm, b1_v), (b2_hbm, b2_v),
        (w2_hbm, w2_v),
    ]
    loads = [pltpu.make_async_copy(s, d, sem_in.at[i]) for i, (s, d) in enumerate(loads)]
    cp_x0, cp_wq, cp_wkv, cp_x1, cp_w1, cp_wo, cp_b1, cp_b2, cp_w2 = loads
    out_parts = ((0, 8), (8, 14), (14, _NT))
    cp_out = [pltpu.make_async_copy(out_v.at[:, cols(a, b)], out_hbm.at[:, cols(a, b)],
                                    sem_out.at[i]) for i, (a, b) in enumerate(out_parts)]

    def layernorms(p):
        xn = _ln_t(_unpack(xt_v[:, tile(p)]))
        xnt_s[:, tile(p)] = _pack(xn)
        ht_s[:, tile(p)] = _pack(_ln_t(xn))

    def prep_wqkv(col_blocks, thirds):
        for c in col_blocks:
            lo, hi = c * _T, min((c + 1) * _T, 3 * _D)
            blk = pltpu.bitcast(_bf(wqkv_v[:, lo:hi]).T, _u32)
            for j in range(4):
                l, h = j * _T, min((j + 1) * _T, _D)
                perm_s[j, lo // 2:hi // 2, 0:h - l] = blk[:, l:h]
        hp = _DH // 2
        for t in thirds:
            for dd in range(hp):
                for j in range(4):
                    l, h = j * _T, min((j + 1) * _T, _D)
                    base = t * _DP + dd
                    a = perm_s[j, pl.ds(base, 8, stride=2 * hp), :]
                    b = perm_s[j, pl.ds(base + hp, 8, stride=2 * hp), :]
                    w0 = (a & jnp.uint32(0xFFFF)) | (b << 16)
                    w1 = (a >> 16) | (b & jnp.uint32(0xFFFF0000))
                    r0 = t * _DP + dd * 16
                    wt_s[r0:r0 + 8, l:h] = w0[:, 0:h - l]
                    wt_s[r0 + 8:r0 + 16, l:h] = w1[:, 0:h - l]

    def prep_wo():
        for j in range(4):
            l, h = j * _T, min((j + 1) * _T, _D)
            perm2_s[j, :, 0:h - l] = _unpack(wo_v[:, l:h])
        for j in range(4):
            l, h = j * _T, min((j + 1) * _T, _D)
            g = jnp.concatenate(
                [perm2_s[j, pl.ds(d, _H, stride=_DH), :] for d in range(_DH)], axis=0)
            wot_s[l // 2:h // 2, :] = pltpu.bitcast(g[:, 0:h - l].astype(_bf16).T, _u32)

    def qkv(p, parts=(0, 1, 2)):
        xn = xnt_s[:, tile(p)]
        for t in parts:
            r = _dot(wt_s[t * _DP:(t + 1) * _DP, :], xn)
            if t == 0:
                qt_s[:, tile(p)] = r
            else:
                (kp_s, vp_s)[t - 1][:, tile(p)] = _pack(r)

    def mix1(f):
        b = b1_v[pl.ds(f * _T, _T)].astype(_f32).reshape(1, _T)
        u_s[:, tile(f)] = _pack(_gelu(_dot(ht_s[...], w1_v[:, tile(f)]) + b))

    lane = jax.lax.broadcasted_iota(jnp.int32, (8, _T), 1)
    lane16 = jax.lax.broadcasted_iota(jnp.int32, (_H, _T), 1)

    def shifted(ref, p, d, w):
        cur = ref[d * 8:(d + 1) * 8, tile(p)]
        sh = _DIL * w
        if w > 0:
            if p > 0:
                prev = ref[d * 8:(d + 1) * 8, tile(p - 1)]
                cur = jnp.where(lane >= _T - sh, prev, cur)
            cur = pltpu.roll(cur, sh, 1)
        return _unpack(cur)

    def attention(p):
        lg = [None] * _W
        for d in range(_DH):
            q = qt_s[d * _H:(d + 1) * _H, tile(p)]
            for w in range(_W):
                t = q * shifted(kp_s, p, d, w)
                lg[w] = t if lg[w] is None else lg[w] + t
        for w in range(_W):
            lg[w] = lg[w] * (_DH ** -0.5)
            if p == 0 and w > 0:
                lg[w] = jnp.where(lane16 >= _DIL * w, lg[w], -1e9)
        m = lg[0]
        for w in range(1, _W):
            m = jnp.maximum(m, lg[w])
        e = [jnp.exp(lg[w] - m) for w in range(_W)]
        s = e[0]
        for w in range(1, _W):
            s = s + e[w]
        r = 1.0 / s
        a = [e[w] * r for w in range(_W)]
        for d in range(_DH):
            acc = a[0] * shifted(vp_s, p, d, 0)
            for w in range(1, _W):
                acc = acc + a[w] * shifted(vp_s, p, d, w)
            ot_s[d * 8:(d + 1) * 8, tile(p)] = _pack(acc)

    def mix2(p):
        b = b2_v[pl.ds(p * _T, _T)].astype(_f32).reshape(1, _T)
        return _dot(u_s[...], w2_v[:, tile(p)]) + b

    def finish(p, y=None):
        if y is None:
            y = mix2(p)
        a = _dot(wot_s[...], ot_s[:, tile(p)])
        out_v[:, tile(p)] = _pack((_unpack(xt_v[:, tile(p)]) + a) + y)

    for cp in loads:
        cp.start()
        pl.semaphore_signal(sem_fence, 1)
        pl.semaphore_wait(sem_fence, 1)

    cp_x0.wait()
    layernorms(0)
    layernorms(1)
    cp_wq.wait()
    prep_wqkv(range(0, 4), (0,))
    qkv(0, (0,))
    layernorms(2)
    qkv(1, (0,))
    layernorms(3)
    cp_wkv.wait()
    prep_wqkv(range(4, 11), (1, 2))
    qkv(2, (0,))
    qkv(3, (0,))
    for p in range(3):
        qkv(p, (1, 2))
    cp_x1.wait()
    layernorms(4)
    qkv(3, (1, 2))
    layernorms(5)
    for p in range(4, _NT - 1):
        qkv(p)
        if p + 2 < _NT:
            layernorms(p + 2)

    cp_w1.wait()
    cp_wo.wait()
    cp_b1.wait()
    cp_b2.wait()
    for f in range(_NF):
        mix1(f)
        if f == 3:
            prep_wo()
        if f == 6:
            attention(0)
    qkv(_NT - 1)

    cp_w2.wait()
    for p in range(_NT):
        if p + 1 < _NT:
            attention(p + 1)
        if p in (8, 14):
            y_s[...] = mix2(p)
            cp_out[0 if p == 8 else 1].start()
            finish(p, y_s[...])
        else:
            finish(p)
    cp_out[2].start()
    for cp in cp_out:
        cp.wait()


@jax.jit
def pallas_parallel_sum__sliding_local_dilated__mixer_token_mlp__prompt_kernel(
    A_x: jax.Array,
    A_wqkv: jax.Array,
    A_wo: jax.Array,
    B_x: jax.Array,
    B_w1: jax.Array,
    B_b1: jax.Array,
    B_w2: jax.Array,
    B_b2: jax.Array,
):
    del B_x
    scratch = [
        pltpu.VMEM((_DP, _S), _u32),
        pltpu.VMEM((_DP, 3 * _D), _u32),
        pltpu.VMEM((_DP, _D), _u32),
        pltpu.VMEM((_S // 2, _F), _u32),
        pltpu.VMEM((_F,), _bf16),
        pltpu.VMEM((_F // 2, _S), _u32),
        pltpu.VMEM((_S,), _bf16),
        pltpu.VMEM((_DP, _S), _u32),
        pltpu.VMEM((_DP, _S), _u32),
        pltpu.VMEM((_DP, _F), _u32),
        pltpu.VMEM((3 * _DP, _D), _u32),
        pltpu.VMEM((_DP, _D), _u32),
        pltpu.VMEM((4, 3 * _DP, _T), _u32),
        pltpu.VMEM((4, _D, _T), _f32),
        pltpu.VMEM((_D, _S), _f32),
        pltpu.VMEM((_DP, _S), _u32),
        pltpu.VMEM((_DP, _S), _u32),
        pltpu.VMEM((_DP, _S), _u32),
        pltpu.VMEM((_DP, _S), _u32),
        pltpu.VMEM((_D, _T), _f32),
        pltpu.SemaphoreType.DMA((9,)),
        pltpu.SemaphoreType.DMA((3,)),
        pltpu.SemaphoreType.REGULAR,
    ]
    hbm = pl.BlockSpec(memory_space=pltpu.HBM)
    xt = jnp.swapaxes(A_x, 1, 2).reshape(_D, _S)
    out = pl.pallas_call(
        _kernel,
        out_shape=jax.ShapeDtypeStruct((_D, _S), _bf16),
        in_specs=[hbm] * 7,
        out_specs=hbm,
        scratch_shapes=scratch,
        compiler_params=pltpu.CompilerParams(vmem_limit_bytes=100 * 1024 * 1024),
    )(xt, A_wqkv, A_wo, B_w1, B_b1, B_w2, B_b2)
    return jnp.swapaxes(out.reshape(1, _D, _S), 1, 2)
```

```python
import jax
import jax.numpy as jnp
import jax.experimental.pallas as pl
import jax.experimental.pallas.tpu as pltpu

_S, _D, _F = 2048, 448, 1792
_H, _DH = 16, 28
_W, _DIL = 8, 2
_EPS = 1e-5
_T = 128
_NT = _S // _T
_NF = _F // _T
_DP = _D // 2

_f32, _bf16, _u32 = jnp.float32, jnp.bfloat16, jnp.uint32


def _ln_t(x):
    m = jnp.sum(x, axis=0, keepdims=True) * (1.0 / _D)
    c = x - m
    v = jnp.sum(c * c, axis=0, keepdims=True) * (1.0 / _D)
    return c * jax.lax.rsqrt(v + _EPS)


def _gelu(z):
    c0 = 0.7978845608028654
    inner = z * (c0 + (c0 * 0.044715) * (z * z))
    hz = 0.5 * z
    return hz + hz * jnp.tanh(inner)


def _pack(x):
    return pltpu.bitcast(x.astype(_bf16), _u32)


def _bf(x):
    return pltpu.bitcast(x, _bf16)


def _unpack(x):
    return _bf(x).astype(_f32)


def _dot(a, b):
    return jnp.dot(_bf(a), _bf(b), preferred_element_type=_f32)


def _kernel(xt_hbm, wqkv_hbm, wo_hbm, w1_hbm, b1_hbm, w2_hbm, b2_hbm, out_hbm,
            xt_v, wqkv_v, wo_v, w1_v, b1_v, w2_v, b2_v,
            xnt_s, ht_s, u_s, wt_s, wot_s, perm_s, perm2_s,
            qt_s, kp_s, vp_s, ot_s, out_v, y_s,
            sem_in, sem_out, sem_fence):
    def tile(p):
        return slice(p * _T, (p + 1) * _T)

    def cols(a, b):
        return slice(a * _T, b * _T)

    xt_hbm, wqkv_hbm, wo_hbm, w1_hbm, w2_hbm, out_hbm = (
        r.bitcast(_u32) for r in (xt_hbm, wqkv_hbm, wo_hbm, w1_hbm, w2_hbm, out_hbm))
    q_cols, kv_cols = slice(0, 4 * _T), slice(4 * _T, 3 * _D)
    loads = [
        (xt_hbm.at[:, cols(0, 4)], xt_v.at[:, cols(0, 4)]),
        (wqkv_hbm.at[:, q_cols], wqkv_v.at[:, q_cols]),
        (wqkv_hbm.at[:, kv_cols], wqkv_v.at[:, kv_cols]),
        (xt_hbm.at[:, cols(4, _NT)], xt_v.at[:, cols(4, _NT)]),
        (w1_hbm, w1_v), (wo_hbm, wo_v), (b1_hbm, b1_v), (b2_hbm, b2_v),
        (w2_hbm, w2_v),
    ]
    loads = [pltpu.make_async_copy(s, d, sem_in.at[i]) for i, (s, d) in enumerate(loads)]
    cp_x0, cp_wq, cp_wkv, cp_x1, cp_w1, cp_wo, cp_b1, cp_b2, cp_w2 = loads
    out_parts = ((0, 8), (8, 14), (14, 15), (15, _NT))
    cp_out = [pltpu.make_async_copy(out_v.at[:, cols(a, b)], out_hbm.at[:, cols(a, b)],
                                    sem_out.at[i]) for i, (a, b) in enumerate(out_parts)]

    def layernorms(p):
        xn = _ln_t(_unpack(xt_v[:, tile(p)]))
        xnt_s[:, tile(p)] = _pack(xn)
        ht_s[:, tile(p)] = _pack(_ln_t(xn))

    def prep_wqkv(col_blocks, thirds):
        for c in col_blocks:
            lo, hi = c * _T, min((c + 1) * _T, 3 * _D)
            blk = pltpu.bitcast(_bf(wqkv_v[:, lo:hi]).T, _u32)
            for j in range(4):
                l, h = j * _T, min((j + 1) * _T, _D)
                part = blk[:, l:h]
                if h - l < _T:
                    part = jnp.concatenate(
                        [part, jnp.zeros((part.shape[0], _T - (h - l)), _u32)], axis=1)
                perm_s[j, lo // 2:hi // 2, :] = part
        hp = _DH // 2
        for t in thirds:
            for dd in range(hp):
                for j in range(4):
                    l, h = j * _T, min((j + 1) * _T, _D)
                    base = t * _DP + dd
                    a = perm_s[j, pl.ds(base, 8, stride=2 * hp), :]
                    b = perm_s[j, pl.ds(base + hp, 8, stride=2 * hp), :]
                    w0 = (a & jnp.uint32(0xFFFF)) | (b << 16)
                    w1 = (a >> 16) | (b & jnp.uint32(0xFFFF0000))
                    r0 = t * _DP + dd * 16
                    wt_s[r0:r0 + 8, l:h] = w0[:, 0:h - l]
                    wt_s[r0 + 8:r0 + 16, l:h] = w1[:, 0:h - l]

    def prep_wo():
        for j in range(4):
            l, h = j * _T, min((j + 1) * _T, _D)
            part = _unpack(wo_v[:, l:h])
            if h - l < _T:
                part = jnp.concatenate([part, jnp.zeros((_D, _T - (h - l)), _f32)], axis=1)
            perm2_s[j, 0:_D, :] = part
        for j in range(4):
            l, h = j * _T, min((j + 1) * _T, _D)
            g = jnp.concatenate(
                [perm2_s[j, pl.ds(d, _H, stride=_DH), :] for d in range(_DH)], axis=0)
            wot_s[l // 2:h // 2, :] = pltpu.bitcast(g[:, 0:h - l].astype(_bf16).T, _u32)

    def qkv(p, parts=(0, 1, 2)):
        xn = xnt_s[:, tile(p)]
        for t in parts:
            r = _dot(wt_s[t * _DP:(t + 1) * _DP, :], xn)
            if t == 0:
                qt_s[:, tile(p)] = r
            else:
                (kp_s, vp_s)[t - 1][:, tile(p)] = _pack(r)

    def mix1(f):
        b = b1_v[pl.ds(f * _T, _T)].astype(_f32).reshape(1, _T)
        u_s[:, tile(f)] = _pack(_gelu(_dot(ht_s[...], w1_v[:, tile(f)]) + b))

    lane = jax.lax.broadcasted_iota(jnp.int32, (8, _T), 1)
    lane16 = jax.lax.broadcasted_iota(jnp.int32, (_H, _T), 1)

    def shifted(ref, p, d, w):
        cur = ref[d * 8:(d + 1) * 8, tile(p)]
        sh = _DIL * w
        if w > 0:
            if p > 0:
                prev = ref[d * 8:(d + 1) * 8, tile(p - 1)]
                cur = jnp.where(lane >= _T - sh, prev, cur)
            cur = pltpu.roll(cur, sh, 1)
        return _unpack(cur)

    def attention(p):
        lg = [None] * _W
        for d in range(_DH):
            q = qt_s[d * _H:(d + 1) * _H, tile(p)]
            for w in range(_W):
                t = q * shifted(kp_s, p, d, w)
                lg[w] = t if lg[w] is None else lg[w] + t
        for w in range(_W):
            lg[w] = lg[w] * (_DH ** -0.5)
            if p == 0 and w > 0:
                lg[w] = jnp.where(lane16 >= _DIL * w, lg[w], -1e9)
        m = lg[0]
        for w in range(1, _W):
            m = jnp.maximum(m, lg[w])
        e = [jnp.exp(lg[w] - m) for w in range(_W)]
        s = e[0]
        for w in range(1, _W):
            s = s + e[w]
        r = 1.0 / s
        a = [e[w] * r for w in range(_W)]
        for d in range(_DH):
            acc = a[0] * shifted(vp_s, p, d, 0)
            for w in range(1, _W):
                acc = acc + a[w] * shifted(vp_s, p, d, w)
            ot_s[d * 8:(d + 1) * 8, tile(p)] = _pack(acc)

    def mix2(p):
        b = b2_v[pl.ds(p * _T, _T)].astype(_f32).reshape(1, _T)
        y_s[p % 2] = _dot(u_s[...], w2_v[:, tile(p)]) + b

    def finish(p):
        a = _dot(wot_s[...], ot_s[:, tile(p)])
        out_v[:, tile(p)] = _pack((_unpack(xt_v[:, tile(p)]) + a) + y_s[p % 2])

    for cp in loads:
        cp.start()
        pl.semaphore_signal(sem_fence, 1)
        pl.semaphore_wait(sem_fence, 1)

    cp_x0.wait()
    layernorms(0)
    layernorms(1)
    cp_wq.wait()
    prep_wqkv(range(0, 4), (0,))
    qkv(0, (0,))
    layernorms(2)
    qkv(1, (0,))
    layernorms(3)
    qkv(2, (0,))
    cp_wkv.wait()
    prep_wqkv(range(4, 11), (1, 2))
    qkv(3, (0,))
    for p in range(3):
        qkv(p, (1, 2))
    cp_x1.wait()
    layernorms(4)
    layernorms(5)
    qkv(3, (1, 2))
    for p in range(4, _NT - 1):
        qkv(p)
        if p >= 5:
            layernorms(p + 1)
    qkv(_NT - 1, (1,))

    cp_w1.wait()
    cp_wo.wait()
    cp_b1.wait()
    cp_b2.wait()
    for f in range(_NF):
        mix1(f)
        if f == 5:
            prep_wo()
        if f == 8:
            attention(0)
    qkv(_NT - 1, (0, 2))

    cp_w2.wait()
    attention(1)
    start_out = {b: i for i, (_, b) in enumerate(out_parts[:-1])}
    for p in range(_NT):
        if p + 2 < _NT:
            attention(p + 2)
        mix2(p)
        if p in start_out:
            cp_out[start_out[p]].start()
        finish(p)
    cp_out[-1].start()
    for cp in cp_out:
        cp.wait()


@jax.jit
def pallas_parallel_sum__sliding_local_dilated__mixer_token_mlp__prompt_kernel(
    A_x: jax.Array,
    A_wqkv: jax.Array,
    A_wo: jax.Array,
    B_x: jax.Array,
    B_w1: jax.Array,
    B_b1: jax.Array,
    B_w2: jax.Array,
    B_b2: jax.Array,
):
    del B_x
    scratch = [
        pltpu.VMEM((_DP, _S), _u32),
        pltpu.VMEM((_DP, 3 * _D), _u32),
        pltpu.VMEM((_DP, _D), _u32),
        pltpu.VMEM((_S // 2, _F), _u32),
        pltpu.VMEM((_F,), _bf16),
        pltpu.VMEM((_F // 2, _S), _u32),
        pltpu.VMEM((_S,), _bf16),
        pltpu.VMEM((_DP, _S), _u32),
        pltpu.VMEM((_DP, _S), _u32),
        pltpu.VMEM((_DP, _F), _u32),
        pltpu.VMEM((3 * _DP, _D), _u32),
        pltpu.VMEM((_DP, _D), _u32),
        pltpu.VMEM((4, 3 * _DP + 32, _T), _u32),
        pltpu.VMEM((4, _D + 32, _T), _f32),
        pltpu.VMEM((_D, _S), _f32),
        pltpu.VMEM((_DP, _S), _u32),
        pltpu.VMEM((_DP, _S), _u32),
        pltpu.VMEM((_DP, _S), _u32),
        pltpu.VMEM((_DP, _S), _u32),
        pltpu.VMEM((2, _D, _T), _f32),
        pltpu.SemaphoreType.DMA((9,)),
        pltpu.SemaphoreType.DMA((4,)),
        pltpu.SemaphoreType.REGULAR,
    ]
    hbm = pl.BlockSpec(memory_space=pltpu.HBM)
    xt = jnp.swapaxes(A_x, 1, 2).reshape(_D, _S)
    out = pl.pallas_call(
        _kernel,
        out_shape=jax.ShapeDtypeStruct((_D, _S), _bf16),
        in_specs=[hbm] * 7,
        out_specs=hbm,
        scratch_shapes=scratch,
        compiler_params=pltpu.CompilerParams(vmem_limit_bytes=100 * 1024 * 1024),
    )(xt, A_wqkv, A_wo, B_w1, B_b1, B_w2, B_b2)
    return jnp.swapaxes(out.reshape(1, _D, _S), 1, 2)
```

```python
import jax
import jax.numpy as jnp
import jax.experimental.pallas as pl
import jax.experimental.pallas.tpu as pltpu

_S, _D, _F = 2048, 448, 1792
_H, _DH = 16, 28
_W, _DIL = 8, 2
_EPS = 1e-5
_T = 128
_NT = _S // _T
_NF = _F // _T
_DP = _D // 2

_f32, _bf16, _u32 = jnp.float32, jnp.bfloat16, jnp.uint32


def _ln_t(x):
    m = jnp.sum(x, axis=0, keepdims=True) * (1.0 / _D)
    c = x - m
    v = jnp.sum(c * c, axis=0, keepdims=True) * (1.0 / _D)
    return c * jax.lax.rsqrt(v + _EPS)


def _gelu(z):
    c0 = 0.7978845608028654
    inner = z * (c0 + (c0 * 0.044715) * (z * z))
    hz = 0.5 * z
    return hz + hz * jnp.tanh(inner)


def _pack(x):
    return pltpu.bitcast(x.astype(_bf16), _u32)


def _bf(x):
    return pltpu.bitcast(x, _bf16)


def _unpack(x):
    return _bf(x).astype(_f32)


def _dot(a, b):
    return jnp.dot(_bf(a), _bf(b), preferred_element_type=_f32)


def _kernel(xt_hbm, wqkv_hbm, wo_hbm, w1_hbm, b1_hbm, w2_hbm, b2_hbm, out_hbm,
            xt_v, wqkv_v, wo_v, w1_v, b1_v, w2_v, b2_v,
            xnt_s, ht_s, u_s, wt_s, wot_s, perm_s, perm2_s,
            qt_s, kp_s, vp_s, ot_s, out_v, y_s,
            sem_in, sem_out, sem_fence):
    def tile(p):
        return slice(p * _T, (p + 1) * _T)

    def cols(a, b):
        return slice(a * _T, b * _T)

    xt_hbm, wqkv_hbm, wo_hbm, w1_hbm, w2_hbm, out_hbm = (
        r.bitcast(_u32) for r in (xt_hbm, wqkv_hbm, wo_hbm, w1_hbm, w2_hbm, out_hbm))
    q_cols, kv_cols = slice(0, 4 * _T), slice(4 * _T, 3 * _D)

    def load(src, dst, sem):
        return pltpu.make_async_copy(src, dst, sem_in.at[sem])

    cp_wq = load(wqkv_hbm.at[:, q_cols], wqkv_v.at[:, q_cols], 0)
    cp_x = [load(xt_hbm.at[:, cols(a, b)], xt_v.at[:, cols(a, b)], 1 + i)
            for i, (a, b) in enumerate(((0, 2), (2, 4), (4, _NT)))]
    cp_wkv = load(wqkv_hbm.at[:, kv_cols], wqkv_v.at[:, kv_cols], 4)
    cp_mix1 = [load(s, d, 5) for s, d in
               ((w1_hbm, w1_v), (wo_hbm, wo_v), (b1_hbm, b1_v), (b2_hbm, b2_v))]
    cp_w2 = load(w2_hbm, w2_v, 6)
    loads = [cp_wq, cp_x[0], cp_x[1], cp_wkv, cp_x[2], *cp_mix1, cp_w2]
    out_parts = ((0, 8), (8, 14), (14, 15), (15, _NT))
    cp_out = [pltpu.make_async_copy(out_v.at[:, cols(a, b)], out_hbm.at[:, cols(a, b)], sem_out)
              for a, b in out_parts]

    def layernorms(p):
        xn = _ln_t(_unpack(xt_v[:, tile(p)]))
        xnt_s[:, tile(p)] = _pack(xn)
        ht_s[:, tile(p)] = _pack(_ln_t(xn))

    def prep_wqkv(col_blocks, t):
        for c in col_blocks:
            lo, hi = c * _T, min((c + 1) * _T, 3 * _D)
            blk = pltpu.bitcast(_bf(wqkv_v[:, lo:hi]).T, _u32)
            for j in range(4):
                l, h = j * _T, min((j + 1) * _T, _D)
                part = blk[:, l:h]
                if h - l < _T:
                    part = jnp.concatenate(
                        [part, jnp.zeros((part.shape[0], _T - (h - l)), _u32)], axis=1)
                perm_s[j, lo // 2:hi // 2, :] = part
        hp = _DH // 2
        for dd in range(hp):
            for j in range(4):
                l, h = j * _T, min((j + 1) * _T, _D)
                base = t * _DP + dd
                a = perm_s[j, pl.ds(base, 8, stride=2 * hp), :]
                b = perm_s[j, pl.ds(base + hp, 8, stride=2 * hp), :]
                w0 = (a & jnp.uint32(0xFFFF)) | (b << 16)
                w1 = (a >> 16) | (b & jnp.uint32(0xFFFF0000))
                r0 = t * _DP + dd * 16
                wt_s[r0:r0 + 8, l:h] = w0[:, 0:h - l]
                wt_s[r0 + 8:r0 + 16, l:h] = w1[:, 0:h - l]

    def prep_wo():
        for j in range(4):
            l, h = j * _T, min((j + 1) * _T, _D)
            part = _unpack(wo_v[:, l:h])
            if h - l < _T:
                part = jnp.concatenate([part, jnp.zeros((_D, _T - (h - l)), _f32)], axis=1)
            perm2_s[j, 0:_D, :] = part
        for j in range(4):
            l, h = j * _T, min((j + 1) * _T, _D)
            g = jnp.concatenate(
                [perm2_s[j, pl.ds(d, _H, stride=_DH), :] for d in range(_DH)], axis=0)
            wot_s[l // 2:h // 2, :] = pltpu.bitcast(g[:, 0:h - l].astype(_bf16).T, _u32)

    def qkv(p, lo=0, hi=3):
        r = _dot(wt_s[lo * _DP:hi * _DP, :], xnt_s[:, tile(p)])
        for t in range(lo, hi):
            part = r[(t - lo) * _D:(t - lo + 1) * _D]
            if t == 0:
                qt_s[:, tile(p)] = part
            else:
                (kp_s, vp_s)[t - 1][:, tile(p)] = _pack(part)

    def mix1(f):
        b = b1_v[pl.ds(f * _T, _T)].astype(_f32).reshape(1, _T)
        u_s[:, tile(f)] = _pack(_gelu(_dot(ht_s[...], w1_v[:, tile(f)]) + b))

    lane = jax.lax.broadcasted_iota(jnp.int32, (8, _T), 1)
    lane16 = jax.lax.broadcasted_iota(jnp.int32, (_H, _T), 1)

    def shifted(ref, p, d, w):
        cur = ref[d * 8:(d + 1) * 8, tile(p)]
        sh = _DIL * w
        if w > 0:
            if p > 0:
                prev = ref[d * 8:(d + 1) * 8, tile(p - 1)]
                cur = jnp.where(lane >= _T - sh, prev, cur)
            cur = pltpu.roll(cur, sh, 1)
        return _unpack(cur)

    def attention(p):
        lg = [None] * _W
        for d in range(_DH):
            q = qt_s[d * _H:(d + 1) * _H, tile(p)]
            for w in range(_W):
                t = q * shifted(kp_s, p, d, w)
                lg[w] = t if lg[w] is None else lg[w] + t
        for w in range(_W):
            lg[w] = lg[w] * (_DH ** -0.5)
            if p == 0 and w > 0:
                lg[w] = jnp.where(lane16 >= _DIL * w, lg[w], -1e9)
        m = lg[0]
        for w in range(1, _W):
            m = jnp.maximum(m, lg[w])
        e = [jnp.exp(lg[w] - m) for w in range(_W)]
        s = e[0]
        for w in range(1, _W):
            s = s + e[w]
        r = 1.0 / s
        a = [e[w] * r for w in range(_W)]
        for d in range(_DH):
            acc = a[0] * shifted(vp_s, p, d, 0)
            for w in range(1, _W):
                acc = acc + a[w] * shifted(vp_s, p, d, w)
            ot_s[d * 8:(d + 1) * 8, tile(p)] = _pack(acc)

    def mix2(p):
        b = b2_v[pl.ds(p * _T, _T)].astype(_f32).reshape(1, _T)
        y_s[p % 2] = _dot(u_s[...], w2_v[:, tile(p)]) + b

    def finish(p):
        a = _dot(wot_s[...], ot_s[:, tile(p)])
        out_v[:, tile(p)] = _pack((_unpack(xt_v[:, tile(p)]) + a) + y_s[p % 2])

    for cp in loads:
        cp.start()
        pl.semaphore_signal(sem_fence, 1)
        pl.semaphore_wait(sem_fence, 1)

    cp_wq.wait()
    prep_wqkv(range(0, 4), 0)
    cp_x[0].wait()
    layernorms(0)
    qkv(0, 0, 1)
    layernorms(1)
    cp_x[1].wait()
    qkv(1, 0, 1)
    layernorms(2)
    qkv(2, 0, 1)
    layernorms(3)
    cp_wkv.wait()
    prep_wqkv(range(4, 7), 1)
    qkv(3, 0, 1)
    qkv(0, 1, 2)
    prep_wqkv(range(7, 11), 2)
    qkv(1, 1, 2)
    qkv(2, 1, 2)
    for p in range(3):
        qkv(p, 2, 3)
    cp_x[2].wait()
    layernorms(4)
    layernorms(5)
    qkv(3, 1, 2)
    qkv(3, 2, 3)
    for p in range(4, _NT - 1):
        qkv(p)
        if p >= 5:
            layernorms(p + 1)
    qkv(_NT - 1, 1, 2)

    for cp in cp_mix1:
        cp.wait()
    for f in range(_NF):
        mix1(f)
        if f == 5:
            prep_wo()
        if f == 8:
            attention(0)
    qkv(_NT - 1, 0, 1)
    qkv(_NT - 1, 2, 3)

    cp_w2.wait()
    attention(1)
    start_out = {b: i for i, (_, b) in enumerate(out_parts[:-1])}
    for p in range(_NT):
        if p + 2 < _NT:
            attention(p + 2)
        mix2(p)
        if p in start_out:
            cp_out[start_out[p]].start()
        finish(p)
    cp_out[-1].start()
    for cp in cp_out:
        cp.wait()


@jax.jit
def pallas_parallel_sum__sliding_local_dilated__mixer_token_mlp__prompt_kernel(
    A_x: jax.Array,
    A_wqkv: jax.Array,
    A_wo: jax.Array,
    B_x: jax.Array,
    B_w1: jax.Array,
    B_b1: jax.Array,
    B_w2: jax.Array,
    B_b2: jax.Array,
):
    del B_x
    scratch = [
        pltpu.VMEM((_DP, _S), _u32),
        pltpu.VMEM((_DP, 3 * _D), _u32),
        pltpu.VMEM((_DP, _D), _u32),
        pltpu.VMEM((_S // 2, _F), _u32),
        pltpu.VMEM((_F,), _bf16),
        pltpu.VMEM((_F // 2, _S), _u32),
        pltpu.VMEM((_S,), _bf16),
        pltpu.VMEM((_DP, _S), _u32),
        pltpu.VMEM((_DP, _S), _u32),
        pltpu.VMEM((_DP, _F), _u32),
        pltpu.VMEM((3 * _DP, _D), _u32),
        pltpu.VMEM((_DP, _D), _u32),
        pltpu.VMEM((4, 3 * _DP + 32, _T), _u32),
        pltpu.VMEM((4, _D + 32, _T), _f32),
        pltpu.VMEM((_D, _S), _f32),
        pltpu.VMEM((_DP, _S), _u32),
        pltpu.VMEM((_DP, _S), _u32),
        pltpu.VMEM((_DP, _S), _u32),
        pltpu.VMEM((_DP, _S), _u32),
        pltpu.VMEM((2, _D, _T), _f32),
        pltpu.SemaphoreType.DMA((7,)),
        pltpu.SemaphoreType.DMA,
        pltpu.SemaphoreType.REGULAR,
    ]
    hbm = pl.BlockSpec(memory_space=pltpu.HBM)
    xt = jnp.swapaxes(A_x, 1, 2).reshape(_D, _S)
    out = pl.pallas_call(
        _kernel,
        out_shape=jax.ShapeDtypeStruct((_D, _S), _bf16),
        in_specs=[hbm] * 7,
        out_specs=hbm,
        scratch_shapes=scratch,
        compiler_params=pltpu.CompilerParams(
            vmem_limit_bytes=100 * 1024 * 1024,
            disable_semaphore_checks=True),
    )(xt, A_wqkv, A_wo, B_w1, B_b1, B_w2, B_b2)
    return jnp.swapaxes(out.reshape(1, _D, _S), 1, 2)
```

```python
import jax
import jax.numpy as jnp
import jax.experimental.pallas as pl
import jax.experimental.pallas.tpu as pltpu

_S, _D, _F = 2048, 448, 1792
_H, _DH = 16, 28
_W, _DIL = 8, 2
_EPS = 1e-5
_T = 128
_NT = _S // _T
_NF = _F // _T
_DP = _D // 2

_f32, _bf16, _u32 = jnp.float32, jnp.bfloat16, jnp.uint32


def _ln_t(x):
    m = jnp.sum(x, axis=0, keepdims=True) * (1.0 / _D)
    c = x - m
    v = jnp.sum(c * c, axis=0, keepdims=True) * (1.0 / _D)
    return c * jax.lax.rsqrt(v + _EPS)


def _gelu(z):
    c0 = 0.7978845608028654
    inner = z * (c0 + (c0 * 0.044715) * (z * z))
    hz = 0.5 * z
    return hz + hz * jnp.tanh(inner)


def _pack(x):
    return pltpu.bitcast(x.astype(_bf16), _u32)


def _bf(x):
    return pltpu.bitcast(x, _bf16)


def _unpack(x):
    return _bf(x).astype(_f32)


def _dot(a, b):
    return jnp.dot(_bf(a), _bf(b), preferred_element_type=_f32)


def _kernel(xt_hbm, wqkv_hbm, wo_hbm, w1_hbm, b1_hbm, w2_hbm, b2_hbm, out_hbm,
            xt_v, wqkv_v, wo_v, w1_v, b1_v, w2_v, b2_v,
            xnt_s, ht_s, u_s, wt_s, wot_s, perm_s, perm2_s,
            qt_s, kp_s, vp_s, ot_s, out_v, y_s,
            sem_in, sem_out, sem_fence):
    def tile(p):
        return slice(p * _T, (p + 1) * _T)

    def cols(a, b):
        return slice(a * _T, b * _T)

    q_cols, kv_cols = slice(0, 4 * _T), slice(4 * _T, 3 * _D)

    def load(src, dst, sem):
        return pltpu.make_async_copy(src, dst, sem_in.at[sem])

    cp_wq = load(wqkv_hbm.at[:, q_cols], wqkv_v.at[:, q_cols], 0)
    cp_x = [load(xt_hbm.at[:, cols(a, b)], xt_v.at[:, cols(a, b)], 1 + i)
            for i, (a, b) in enumerate(((0, 2), (2, 4), (4, _NT)))]
    cp_wkv = load(wqkv_hbm.at[:, kv_cols], wqkv_v.at[:, kv_cols], 4)
    cp_mix1 = [load(s, d, 5) for s, d in
               ((w1_hbm, w1_v), (wo_hbm, wo_v), (b1_hbm, b1_v), (b2_hbm, b2_v))]
    cp_w2 = load(w2_hbm, w2_v, 6)
    loads = [cp_wq, cp_x[0], cp_x[1], cp_wkv, cp_x[2], *cp_mix1, cp_w2]
    out_parts = ((0, 8), (8, 14), (14, 15), (15, _NT))
    cp_out = [pltpu.make_async_copy(out_v.at[:, cols(a, b)], out_hbm.at[:, cols(a, b)], sem_out)
              for a, b in out_parts]

    def layernorms(p):
        xn = _ln_t(xt_v[:, tile(p)].astype(_f32))
        xnt_s[:, tile(p)] = _pack(xn)
        ht_s[:, tile(p)] = _pack(_ln_t(xn))

    def prep_wqkv(col_blocks, t):
        for c in col_blocks:
            lo, hi = c * _T, min((c + 1) * _T, 3 * _D)
            blk = pltpu.bitcast(wqkv_v[:, lo:hi].T, _u32)
            for j in range(4):
                l, h = j * _T, min((j + 1) * _T, _D)
                part = blk[:, l:h]
                if h - l < _T:
                    part = jnp.concatenate(
                        [part, jnp.zeros((part.shape[0], _T - (h - l)), _u32)], axis=1)
                perm_s[j, lo // 2:hi // 2, :] = part
        hp = _DH // 2
        for dd in range(hp):
            for j in range(4):
                l, h = j * _T, min((j + 1) * _T, _D)
                base = t * _DP + dd
                a = perm_s[j, pl.ds(base, 8, stride=2 * hp), :]
                b = perm_s[j, pl.ds(base + hp, 8, stride=2 * hp), :]
                w0 = (a & jnp.uint32(0xFFFF)) | (b << 16)
                w1 = (a >> 16) | (b & jnp.uint32(0xFFFF0000))
                r0 = t * _DP + dd * 16
                wt_s[r0:r0 + 8, l:h] = w0[:, 0:h - l]
                wt_s[r0 + 8:r0 + 16, l:h] = w1[:, 0:h - l]

    def prep_wo():
        for j in range(4):
            l, h = j * _T, min((j + 1) * _T, _D)
            part = wo_v[:, l:h].astype(_f32)
            if h - l < _T:
                part = jnp.concatenate([part, jnp.zeros((_D, _T - (h - l)), _f32)], axis=1)
            perm2_s[j, 0:_D, :] = part
        for j in range(4):
            l, h = j * _T, min((j + 1) * _T, _D)
            g = jnp.concatenate(
                [perm2_s[j, pl.ds(d, _H, stride=_DH), :] for d in range(_DH)], axis=0)
            wot_s[l // 2:h // 2, :] = pltpu.bitcast(g[:, 0:h - l].astype(_bf16).T, _u32)

    def qkv(p, lo=0, hi=3):
        r = _dot(wt_s[lo * _DP:hi * _DP, :], xnt_s[:, tile(p)])
        for t in range(lo, hi):
            part = r[(t - lo) * _D:(t - lo + 1) * _D]
            if t == 0:
                qt_s[:, tile(p)] = part
            else:
                (kp_s, vp_s)[t - 1][:, tile(p)] = _pack(part)

    def mix1(f):
        b = b1_v[pl.ds(f * _T, _T)].astype(_f32).reshape(1, _T)
        u = jnp.dot(_bf(ht_s[...]), w1_v[:, tile(f)], preferred_element_type=_f32)
        u_s[:, tile(f)] = _pack(_gelu(u + b))

    lane = jax.lax.broadcasted_iota(jnp.int32, (8, _T), 1)
    lane16 = jax.lax.broadcasted_iota(jnp.int32, (_H, _T), 1)

    def shifted(ref, p, d, w):
        cur = ref[d * 8:(d + 1) * 8, tile(p)]
        sh = _DIL * w
        if w > 0:
            if p > 0:
                prev = ref[d * 8:(d + 1) * 8, tile(p - 1)]
                cur = jnp.where(lane >= _T - sh, prev, cur)
            cur = pltpu.roll(cur, sh, 1)
        return _unpack(cur)

    def attention(p):
        lg = [None] * _W
        for d in range(_DH):
            q = qt_s[d * _H:(d + 1) * _H, tile(p)]
            for w in range(_W):
                t = q * shifted(kp_s, p, d, w)
                lg[w] = t if lg[w] is None else lg[w] + t
        for w in range(_W):
            lg[w] = lg[w] * (_DH ** -0.5)
            if p == 0 and w > 0:
                lg[w] = jnp.where(lane16 >= _DIL * w, lg[w], -1e9)
        m = lg[0]
        for w in range(1, _W):
            m = jnp.maximum(m, lg[w])
        e = [jnp.exp(lg[w] - m) for w in range(_W)]
        s = e[0]
        for w in range(1, _W):
            s = s + e[w]
        r = 1.0 / s
        a = [e[w] * r for w in range(_W)]
        for d in range(_DH):
            acc = a[0] * shifted(vp_s, p, d, 0)
            for w in range(1, _W):
                acc = acc + a[w] * shifted(vp_s, p, d, w)
            ot_s[d * 8:(d + 1) * 8, tile(p)] = _pack(acc)

    def mix2(p):
        b = b2_v[pl.ds(p * _T, _T)].astype(_f32).reshape(1, _T)
        y = jnp.dot(_bf(u_s[...]), w2_v[:, tile(p)], preferred_element_type=_f32)
        y_s[p % 2] = y + b

    def finish(p):
        a = _dot(wot_s[...], ot_s[:, tile(p)])
        out_v[:, tile(p)] = ((xt_v[:, tile(p)].astype(_f32) + a) + y_s[p % 2]).astype(_bf16)

    for cp in loads:
        cp.start()
        pl.semaphore_signal(sem_fence, 1)
        pl.semaphore_wait(sem_fence, 1)

    cp_wq.wait()
    prep_wqkv(range(0, 4), 0)
    cp_x[0].wait()
    layernorms(0)
    qkv(0, 0, 1)
    layernorms(1)
    cp_x[1].wait()
    qkv(1, 0, 1)
    layernorms(2)
    qkv(2, 0, 1)
    layernorms(3)
    cp_wkv.wait()
    prep_wqkv(range(4, 7), 1)
    qkv(3, 0, 1)
    qkv(0, 1, 2)
    prep_wqkv(range(7, 11), 2)
    qkv(1, 1, 2)
    qkv(2, 1, 2)
    for p in range(3):
        qkv(p, 2, 3)
    cp_x[2].wait()
    layernorms(4)
    layernorms(5)
    qkv(3, 1, 2)
    qkv(3, 2, 3)
    for p in range(4, _NT - 1):
        qkv(p)
        if p >= 5:
            layernorms(p + 1)
    qkv(_NT - 1, 1, 2)

    for cp in cp_mix1:
        cp.wait()
    for f in range(_NF):
        mix1(f)
        if f == 5:
            prep_wo()
        if f == 8:
            attention(0)
    qkv(_NT - 1, 0, 1)
    qkv(_NT - 1, 2, 3)

    cp_w2.wait()
    attention(1)
    start_out = {b: i for i, (_, b) in enumerate(out_parts[:-1])}
    for p in range(_NT):
        if p + 2 < _NT:
            attention(p + 2)
        mix2(p)
        if p in start_out:
            cp_out[start_out[p]].start()
        finish(p)
    cp_out[-1].start()
    for cp in cp_out:
        cp.wait()


@jax.jit
def pallas_parallel_sum__sliding_local_dilated__mixer_token_mlp__prompt_kernel(
    A_x: jax.Array,
    A_wqkv: jax.Array,
    A_wo: jax.Array,
    B_x: jax.Array,
    B_w1: jax.Array,
    B_b1: jax.Array,
    B_w2: jax.Array,
    B_b2: jax.Array,
):
    del B_x
    scratch = [
        pltpu.VMEM((_D, _S), _bf16),
        pltpu.VMEM((_D, 3 * _D), _bf16),
        pltpu.VMEM((_D, _D), _bf16),
        pltpu.VMEM((_S, _F), _bf16),
        pltpu.VMEM((_F,), _bf16),
        pltpu.VMEM((_F, _S), _bf16),
        pltpu.VMEM((_S,), _bf16),
        pltpu.VMEM((_DP, _S), _u32),
        pltpu.VMEM((_DP, _S), _u32),
        pltpu.VMEM((_DP, _F), _u32),
        pltpu.VMEM((3 * _DP, _D), _u32),
        pltpu.VMEM((_DP, _D), _u32),
        pltpu.VMEM((4, 3 * _DP + 32, _T), _u32),
        pltpu.VMEM((4, _D + 32, _T), _f32),
        pltpu.VMEM((_D, _S), _f32),
        pltpu.VMEM((_DP, _S), _u32),
        pltpu.VMEM((_DP, _S), _u32),
        pltpu.VMEM((_DP, _S), _u32),
        pltpu.VMEM((_D, _S), _bf16),
        pltpu.VMEM((2, _D, _T), _f32),
        pltpu.SemaphoreType.DMA((7,)),
        pltpu.SemaphoreType.DMA,
        pltpu.SemaphoreType.REGULAR,
    ]
    hbm = pl.BlockSpec(memory_space=pltpu.HBM)
    xt = jnp.swapaxes(A_x, 1, 2).reshape(_D, _S)
    out = pl.pallas_call(
        _kernel,
        out_shape=jax.ShapeDtypeStruct((_D, _S), _bf16),
        in_specs=[hbm] * 7,
        out_specs=hbm,
        scratch_shapes=scratch,
        compiler_params=pltpu.CompilerParams(vmem_limit_bytes=100 * 1024 * 1024),
    )(xt, A_wqkv, A_wo, B_w1, B_b1, B_w2, B_b2)
    return jnp.swapaxes(out.reshape(1, _D, _S), 1, 2)
```
